```python
import os as _os
_os.environ.setdefault("JAX_PLATFORMS", "cpu")
import jax
import jax.numpy as jnp

def _softmax(x, axis=-1):
    return jax.nn.softmax(x, axis=axis)
def _gelu(x):
    return jax.nn.gelu(x, approximate=True)
def _silu(x):
    return jax.nn.silu(x)
def _sigmoid(x):
    return jax.nn.sigmoid(x)
def _layernorm(x, axis=-1, eps=1e-5):
    m = jnp.mean(x, axis=axis, keepdims=True)
    v = jnp.var(x, axis=axis, keepdims=True)
    return (x - m) / jnp.sqrt(v + eps)
def _scatter_add(tgt, idx, src, axis=0):
    return tgt.at[idx].add(src)
def _segment_sum(src, seg, n):
    return jax.ops.segment_sum(src, seg, n)
class _Rng:
    def __init__(self, key):
        self._k = key
    def _next(self):
        self._k, sub = jax.random.split(self._k)
        return sub
    def normal(self, shape):
        return jax.random.normal(self._next(), shape, dtype=jnp.bfloat16)
    def randint(self, lo, hi, shape):
        return jax.random.randint(self._next(), shape, lo, hi, dtype=jnp.int32)
    def uniform(self, shape, lo=0.0, hi=1.0):
        return jax.random.uniform(self._next(), shape, jnp.bfloat16, lo, hi)
    def permutation(self, n):
        return jax.random.permutation(self._next(), n)


kernel_name = 'concat_heads__gqa_block_cached__gqa_block_cached__near_ridge'

def setup_inputs():
    _rng = _Rng(jax.random.key(int.from_bytes(__import__("os").urandom(4), "little")))
    _w = (lambda a: (lambda t: t.astype(jnp.bfloat16) if jnp.issubdtype(t.dtype, jnp.floating) else t)(jnp.asarray(a)))
    def _A_setup():
        B, Sq, D = 8, 128, 576
        Hq, Hkv, Sk, Dh = 32, 16, 512, 128
        assert Hq % Hkv == 0, (Hq, Hkv)
        return {
            "x": _w((lambda *s: _rng.normal(s) * 0.8)(B, Sq, D)),
            "k_cache": _w((lambda *s: _rng.normal(s) * 0.8)(B, Hkv, Sk, Dh)),
            "v_cache": _w((lambda *s: _rng.normal(s) * 0.05)(B, Hkv, Sk, Dh)),
            "wq": _w((lambda *s: _rng.normal(s) * 0.8)(D, Hq * Dh) * (D ** -0.5)),
            "wo": _w((lambda *s: _rng.normal(s) * 0.05)(Hq * Dh, D) * ((Hq * Dh) ** -0.5)),
        }
    _A_in = _A_setup()

    def _B_setup():
        B, Sq, D = 8, 128, 576
        Hq, Hkv, Sk, Dh = 32, 16, 512, 128
        assert Hq % Hkv == 0, (Hq, Hkv)
        return {
            "x": _w((lambda *s: _rng.normal(s) * 0.8)(B, Sq, D)),
            "k_cache": _w((lambda *s: _rng.normal(s) * 0.8)(B, Hkv, Sk, Dh)),
            "v_cache": _w((lambda *s: _rng.normal(s) * 0.05)(B, Hkv, Sk, Dh)),
            "wq": _w((lambda *s: _rng.normal(s) * 0.8)(D, Hq * Dh) * (D ** -0.5)),
            "wo": _w((lambda *s: _rng.normal(s) * 0.05)(Hq * Dh, D) * ((Hq * Dh) ** -0.5)),
        }
    _B_in = _B_setup()

    return {
        "A_x": _A_in["x"],
        "A_k_cache": _A_in["k_cache"],
        "A_v_cache": _A_in["v_cache"],
        "A_wq": _A_in["wq"],
        "A_wo": _A_in["wo"],
        "B_x": _B_in["x"],
        "B_k_cache": _B_in["k_cache"],
        "B_v_cache": _B_in["v_cache"],
        "B_wq": _B_in["wq"],
        "B_wo": _B_in["wo"],
    }

def reference(A_x, A_k_cache, A_v_cache, A_wq, A_wo, B_x, B_k_cache, B_v_cache, B_wq, B_wo):
    def _A_ref(x, k_cache, v_cache, wq, wo):
        B, Sq, D = x.shape
        Hq, Dh = 32, 128
        Hkv = k_cache.shape[1]
        rep = Hq // Hkv
        q = (lambda x, *d: x.transpose(*d))((x @ wq).reshape(B, Sq, Hq, Dh), 0, 2, 1, 3)
        k = jnp.repeat(k_cache, rep, axis=1)
        v = jnp.repeat(v_cache, rep, axis=1)
        scores = jnp.einsum("bhqd,bhkd->bhqk", q, k) * (Dh ** -0.5)
        p = _softmax(scores, axis=-1)
        o = jnp.einsum("bhqk,bhkd->bhqd", p, v)
        return (lambda x, *d: x.transpose(*d))(o, 0, 2, 1, 3).reshape(B, Sq, Hq * Dh) @ wo

    def _B_ref(x, k_cache, v_cache, wq, wo):
        B, Sq, D = x.shape
        Hq, Dh = 32, 128
        Hkv = k_cache.shape[1]
        rep = Hq // Hkv
        q = (lambda x, *d: x.transpose(*d))((x @ wq).reshape(B, Sq, Hq, Dh), 0, 2, 1, 3)
        k = jnp.repeat(k_cache, rep, axis=1)
        v = jnp.repeat(v_cache, rep, axis=1)
        scores = jnp.einsum("bhqd,bhkd->bhqk", q, k) * (Dh ** -0.5)
        p = _softmax(scores, axis=-1)
        o = jnp.einsum("bhqk,bhkd->bhqd", p, v)
        return (lambda x, *d: x.transpose(*d))(o, 0, 2, 1, 3).reshape(B, Sq, Hq * Dh) @ wo

    a = _A_ref(A_x, A_k_cache, A_v_cache, A_wq, A_wo)
    b = _B_ref(B_x, B_k_cache, B_v_cache, B_wq, B_wo)
    return jnp.concatenate([a, b], axis=-1)
```

```python
import jax
import jax.numpy as jnp
from jax import lax
import jax.experimental.pallas as pl
import jax.experimental.pallas.tpu as pltpu
import numpy as np

B, SQ, D = 8, 128, 576
HQ, HKV, SK, DH = 32, 16, 512, 128
M = B * SQ
HD = HQ * DH
P1_NC = 512
P1_MC = 1024
P2_U = 4
P2_MODE = "skew1"
P3_MC = 512
SCALE = float(DH ** -0.5 * np.log2(np.e))
NQC = HD // P1_NC
NOC = M // P3_MC


def _attn_units(q_buf, o_buf, k_buf, v_buf, b, j0, nu):
    rows = pl.ds(pl.multiple_of(b * SQ, SQ), SQ)

    def cols(u, h):
        return pl.ds(pl.multiple_of((j0 + u) * 256 + h * 128, 128), 128)

    def qk(u):
        q = jnp.concatenate([q_buf[rows, cols(u, 0)], q_buf[rows, cols(u, 1)]], axis=0)
        k = k_buf[b, j0 + u]
        return lax.dot_general(q, k, (((1,), (1,)), ((), ())), preferred_element_type=jnp.float32)

    def sm(s):
        m = jnp.max(s, axis=1, keepdims=True)
        p = jnp.exp2(s - m)
        l = jnp.sum(p, axis=1, keepdims=True)
        return p.astype(jnp.bfloat16), l

    def pv(u, p, l):
        v = v_buf[b, j0 + u]
        o = jnp.dot(p, v, preferred_element_type=jnp.float32)
        o = (o * pl.reciprocal(l, approx=False)).astype(jnp.bfloat16)
        o_buf[rows, cols(u, 0)] = o[:SQ]
        o_buf[rows, cols(u, 1)] = o[SQ:]

    if P2_MODE == "plain":
        for u in range(nu):
            p, l = sm(qk(u))
            pv(u, p, l)
    elif P2_MODE == "skew1":
        s = qk(0)
        for u in range(nu):
            s_next = qk(u + 1) if u + 1 < nu else None
            p, l = sm(s)
            pv(u, p, l)
            s = s_next
    elif P2_MODE == "skew2":
        p, l = sm(qk(0))
        for u in range(nu):
            if u + 1 < nu:
                nxt = sm(qk(u + 1))
            pv(u, p, l)
            if u + 1 < nu:
                p, l = nxt


def _kernel(xa, ka, va, wqa, woa, xb, kb, vb, wqb, wob, out_hbm,
            xt_buf, x_buf, wq_buf, wo_buf, k_buf, v_buf, q_buf, o_buf, outt_buf, out_buf,
            sem_x, sem_wq, sem_wo, sem_k, sem_v, sem_out):
    xs, ks, vs, wqs, wos = (xa, xb), (ka, kb), (va, vb), (wqa, wqb), (woa, wob)

    def x_cp(br):
        return pltpu.make_async_copy(xs[br], xt_buf.at[br], sem_x.at[br])

    def wq_cp(br, c):
        return pltpu.make_async_copy(wqs[br].at[:, pl.ds(c * P1_NC, P1_NC)],
                                     wq_buf.at[br, :, pl.ds(c * P1_NC, P1_NC)], sem_wq.at[br, c])

    def wo_cp(br):
        return pltpu.make_async_copy(wos[br], wo_buf.at[br], sem_wo.at[br])

    def k_cp(br, b):
        return pltpu.make_async_copy(ks[br].at[b], k_buf.at[b], sem_k.at[b])

    def v_cp(br, b):
        return pltpu.make_async_copy(vs[br].at[b], v_buf.at[b], sem_v.at[b])

    def out_cp(c):
        return pltpu.make_async_copy(out_buf.at[pl.ds(c * P3_MC, P3_MC)],
                                     out_hbm.at[pl.ds(c * P3_MC, P3_MC)], sem_out.at[c])

    x_cp(0).start()
    wq_cp(0, 0).start()
    wq_cp(0, 1).start()

    for br in range(2):
        x_cp(br).wait()
        for b in range(B):
            x_buf[pl.ds(b * SQ, SQ), :] = xt_buf[br, b].T
        for c in range(NQC):
            if br == 0:
                if c + 2 < NQC:
                    wq_cp(0, c + 2).start()
                if c >= NQC - 3:
                    bb = c - (NQC - 3)
                    k_cp(0, bb).start(); v_cp(0, bb).start()
            wq_cp(br, c).wait()
            for mi in range(M // P1_MC):
                xm = x_buf[pl.ds(mi * P1_MC, P1_MC), :]
                w = wq_buf[br, :, pl.ds(c * P1_NC, P1_NC)]
                q = jnp.dot(xm, w, preferred_element_type=jnp.float32) * SCALE
                q_buf[pl.ds(mi * P1_MC, P1_MC), pl.ds(c * P1_NC, P1_NC)] = q.astype(jnp.bfloat16)

        for b in range(B):
            if br == 0:
                if b + 3 < B:
                    k_cp(0, b + 3).start(); v_cp(0, b + 3).start()
                if b == 5:
                    wo_cp(0).start()
                if b == 6:
                    x_cp(1).start()
                    for c in range(NQC):
                        wq_cp(1, c).start()
            k_cp(br, b).wait()
            v_cp(br, b).wait()
            if P2_U == HKV:
                _attn_units(q_buf, o_buf, k_buf, v_buf, b, 0, HKV)
            else:
                def unit(jj, carry, b=b):
                    _attn_units(q_buf, o_buf, k_buf, v_buf, b, jj * P2_U, P2_U)
                    return carry
                lax.fori_loop(0, HKV // P2_U, unit, 0)
            if br == 0 and b >= 6:
                pass

        if br == 0:
            for b in range(B):
                k_cp(1, b).start(); v_cp(1, b).start()
            wo_cp(1).start()
        wo_cp(br).wait()
        for c in range(NOC):
            o = o_buf[pl.ds(c * P3_MC, P3_MC), :]
            r = lax.dot_general(wo_buf[br], o, (((1,), (1,)), ((), ())), preferred_element_type=jnp.float32)
            outt_buf[pl.ds(br * D, D), pl.ds(c * P3_MC, P3_MC)] = r.astype(jnp.bfloat16)
            if br == 1:
                for bb in range(P3_MC // SQ):
                    r0 = c * P3_MC + bb * SQ
                    out_buf[pl.ds(r0, SQ), :] = outt_buf[:, pl.ds(r0, SQ)].T
                out_cp(c).start()
    for c in range(NOC):
        out_cp(c).wait()


@jax.jit
def pallas_concat_heads__gqa_block_cached__gqa_block_cached__near_ridge_kernel(
        A_x, A_k_cache, A_v_cache, A_wq, A_wo, B_x, B_k_cache, B_v_cache, B_wq, B_wo):
    any_spec = pl.BlockSpec(memory_space=pl.ANY)
    out = pl.pallas_call(
        _kernel,
        out_shape=jax.ShapeDtypeStruct((M, 2 * D), jnp.bfloat16),
        in_specs=[any_spec] * 10,
        out_specs=any_spec,
        scratch_shapes=[
            pltpu.VMEM((2, B, D, SQ), jnp.bfloat16),
            pltpu.VMEM((M, D), jnp.bfloat16),
            pltpu.VMEM((2, D, HD), jnp.bfloat16),
            pltpu.VMEM((2, D, HD), jnp.bfloat16),
            pltpu.VMEM((B, HKV, SK, DH), jnp.bfloat16),
            pltpu.VMEM((B, HKV, SK, DH), jnp.bfloat16),
            pltpu.VMEM((M, HD), jnp.bfloat16),
            pltpu.VMEM((M, HD), jnp.bfloat16),
            pltpu.VMEM((2 * D, M), jnp.bfloat16),
            pltpu.VMEM((M, 2 * D), jnp.bfloat16),
            pltpu.SemaphoreType.DMA((2,)),
            pltpu.SemaphoreType.DMA((2, NQC)),
            pltpu.SemaphoreType.DMA((2,)),
            pltpu.SemaphoreType.DMA((B,)),
            pltpu.SemaphoreType.DMA((B,)),
            pltpu.SemaphoreType.DMA((NOC,)),
        ],
        compiler_params=pltpu.CompilerParams(vmem_limit_bytes=100 * 1024 * 1024),
    )(jnp.swapaxes(A_x, 1, 2), A_k_cache, A_v_cache, A_wq, A_wo.T,
      jnp.swapaxes(B_x, 1, 2), B_k_cache, B_v_cache, B_wq, B_wo.T)
    return out.reshape(B, SQ, 2 * D)
```

```python
import jax
import jax.numpy as jnp
from jax import lax
import jax.experimental.pallas as pl
import jax.experimental.pallas.tpu as pltpu
import numpy as np

B, SQ, D = 8, 128, 576
HQ, HKV, SK, DH = 32, 16, 512, 128
M = B * SQ
HD = HQ * DH

P1_NC = 512
P1_LC = 1024
P2_NB = 4
P2_G = 16
P3_MC = 256
N1, N2, N3 = HD // P1_LC, B // P2_NB, M // P3_MC
XS0 = (0, 4, B)
WQ0 = (0, 512, P1_LC)
SCALE = float(DH ** -0.5 * np.log2(np.e))


def _mo(x, n):
    return x if isinstance(x, int) else pl.multiple_of(x, n)


def _attention(q_buf, o_buf, k_buf, v_buf, br, b0):
    units = [(b0 + i, j) for i in range(P2_NB) for j in range(HKV)]

    def scores(b, j):
        rows = pl.ds(_mo(b * SQ, SQ), SQ)
        q = jnp.concatenate([q_buf[rows, pl.ds(j * 2 * DH, DH)],
                             q_buf[rows, pl.ds(j * 2 * DH + DH, DH)]], axis=0)
        return lax.dot_general(q, k_buf[br, b, j], (((1,), (1,)), ((), ())),
                               preferred_element_type=jnp.float32)

    def softmax_numerator(s):
        m = jnp.max(s, axis=1, keepdims=True)
        p = jnp.exp2(s - m)
        p16 = p.astype(jnp.bfloat16)
        return p16, jnp.sum(p, axis=1, keepdims=True)

    def weighted_values(b, j, p, l):
        rows = pl.ds(_mo(b * SQ, SQ), SQ)
        o = jnp.dot(p, v_buf[br, b, j], preferred_element_type=jnp.float32)
        r = pltpu.reciprocal(l, approx=True)
        r = r * (2.0 - l * r)
        o = (o * r).astype(jnp.bfloat16)
        o_buf[rows, pl.ds(j * 2 * DH, DH)] = o[:SQ]
        o_buf[rows, pl.ds(j * 2 * DH + DH, DH)] = o[SQ:]

    for u in range(0, len(units), P2_G):
        group = units[u:u + P2_G]
        ss = [scores(*x) for x in group]
        ps = [softmax_numerator(s) for s in ss]
        for x, (p, l) in zip(group, ps):
            weighted_values(*x, p, l)


def _kernel(xa, ka, va, wqa, woa, xb, kb, vb, wqb, wob, out_hbm,
            xt_buf, x_buf, wq_buf, wo_buf, k_buf, v_buf, q_buf, o_buf, outt_buf, out_buf,
            sem_x, sem_wq0, sem_wq, sem_wo, sem_k, sem_v, sem_out):
    xs, ks, vs, wqs, wos = (xa, xb), (ka, kb), (va, vb), (wqa, wqb), (woa, wob)

    def x_cp(br, i):
        sp = XS0 if br == 0 else (0, B)
        sl = pl.ds(sp[i], sp[i + 1] - sp[i])
        return pltpu.make_async_copy(xs[br].at[sl], xt_buf.at[br, sl], sem_x.at[br, i])

    def wq0_cp(i):
        sl = pl.ds(WQ0[i], WQ0[i + 1] - WQ0[i])
        return pltpu.make_async_copy(wqs[0].at[:, sl], wq_buf.at[0, :, sl], sem_wq0.at[i])

    def wq_cp(br, c):
        sl = pl.ds(_mo(c * P1_LC, P1_LC), P1_LC)
        return pltpu.make_async_copy(wqs[br].at[:, sl], wq_buf.at[br, :, sl], sem_wq.at[br, c])

    def wo_cp(br):
        return pltpu.make_async_copy(wos[br], wo_buf.at[br], sem_wo.at[br])

    def k_cp(br, g):
        sl = pl.ds(g * P2_NB, P2_NB)
        return pltpu.make_async_copy(ks[br].at[sl], k_buf.at[br, sl], sem_k.at[br, g])

    def v_cp(br, g):
        sl = pl.ds(g * P2_NB, P2_NB)
        return pltpu.make_async_copy(vs[br].at[sl], v_buf.at[br, sl], sem_v.at[br, g])

    def out_cp(br, c):
        rows = pl.ds(_mo(c * P3_MC, P3_MC), P3_MC)
        cols = pl.ds(0, 512) if br == 0 else pl.ds(512, 640)
        return pltpu.make_async_copy(out_buf.at[rows, cols], out_hbm.at[rows, cols],
                                     sem_out.at[br, c])

    def per_branch(br, fn):
        pl.when(br == 0)(lambda: fn(0))
        pl.when(br == 1)(lambda: fn(1))

    def transpose_x(src, b0, nb):
        for i in range(nb):
            x_buf[pl.ds(_mo((b0 + i) * SQ, SQ), SQ), :] = xt_buf[src, b0 + i].T

    def q_proj(br, r0, r1, c0, n):
        for c in range(0, n, P1_NC):
            cols = pl.ds(_mo(c0 + c, 128), min(P1_NC, n - c))
            q = jnp.dot(x_buf[pl.ds(r0, r1 - r0), :], wq_buf[br, :, cols],
                        preferred_element_type=jnp.float32) * SCALE
            q_buf[pl.ds(r0, r1 - r0), cols] = q.astype(jnp.bfloat16)

    def out_proj(br, c):
        rows = pl.ds(_mo(c * P3_MC, P3_MC), P3_MC)
        res = lax.dot_general(wo_buf[br], o_buf[rows, :], (((1,), (1,)), ((), ())),
                              preferred_element_type=jnp.float32)
        outt_buf[pl.ds(_mo(br * D, 64), D), rows] = res.astype(jnp.bfloat16)

    def transpose_out(br, c):
        feats = pl.ds(_mo(br * 512, 512), 640)
        for i in range(P3_MC // SQ):
            rows = pl.ds(_mo(c * P3_MC + i * SQ, SQ), SQ)
            out_buf[rows, feats] = outt_buf[feats, rows].T

    def start_in_order(copies):
        def body(i, carry):
            for k, cp in enumerate(copies):
                pl.when(i == k)(cp.start)
            return carry
        lax.fori_loop(0, len(copies), body, 0)

    def start_range(lo, hi, *makers):
        def body(i, carry):
            for make in makers:
                make(i).start()
            return carry
        lax.fori_loop(lo, hi, body, 0)

    def start_up():
        start_in_order([x_cp(0, 0), wq0_cp(0), x_cp(0, 1), wq0_cp(1)])
        start_range(1, N1, lambda c: wq_cp(0, c))
        start_range(0, N2, lambda g: k_cp(0, g), lambda g: v_cp(0, g))
        start_in_order([wo_cp(0), x_cp(1, 0)])
        start_range(0, N1, lambda c: wq_cp(1, c))
        start_range(0, N2, lambda g: k_cp(1, g), lambda g: v_cp(1, g))
        wo_cp(1).start()
        outt_buf[pl.ds(D, 64), :] = jnp.zeros((64, M), jnp.bfloat16)
        outt_buf[pl.ds(0, D), pl.ds(0, P3_MC)] = jnp.zeros((D, P3_MC), jnp.bfloat16)
        x_cp(0, 0).wait()
        transpose_x(0, XS0[0], XS0[1] - XS0[0])
        wq0_cp(0).wait()
        q_proj(0, 0, XS0[1] * SQ, WQ0[0], WQ0[1] - WQ0[0])
        x_cp(0, 1).wait()
        transpose_x(0, XS0[1], XS0[2] - XS0[1])
        q_proj(0, XS0[1] * SQ, M, WQ0[0], WQ0[1] - WQ0[0])
        wq0_cp(1).wait()
        q_proj(0, 0, M, WQ0[1], WQ0[2] - WQ0[1])

    def branch(br, carry):
        pl.when(br == 0)(start_up)

        def q_trip(c, carry):
            per_branch(br, lambda s: wq_cp(s, c).wait())
            q_proj(br, 0, M, c * P1_LC, P1_LC)
            return carry
        lax.fori_loop(1 - br, N1, q_trip, 0)

        def attn_trip(g, carry):
            def wait_kv(s):
                k_cp(s, g).wait()
                v_cp(s, g).wait()
            per_branch(br, wait_kv)
            _attention(q_buf, o_buf, k_buf, v_buf, br, g * P2_NB)
            return carry
        lax.fori_loop(0, N2, attn_trip, 0)

        per_branch(br, lambda s: wo_cp(s).wait())
        pl.when(br == 0)(lambda: x_cp(1, 0).wait())

        def out_trip(c, carry):
            prev = jnp.maximum(br * N3 + c - 1, 0)
            pbr, pc = prev // N3, prev % N3
            transpose_out(pbr, pc)
            transpose_x(1, c * (B // N3), B // N3)
            out_proj(br, c)
            pl.when(jnp.logical_and(pbr == 0, br + c > 0))(lambda: out_cp(0, pc).start())
            pl.when(pbr == 1)(lambda: out_cp(1, pc).start())
            return carry
        lax.fori_loop(0, N3, out_trip, 0)

        @pl.when(br == 1)
        def _():
            transpose_out(1, N3 - 1)
            out_cp(1, N3 - 1).start()
            for c in range(N3):
                out_cp(0, c).wait()
                out_cp(1, c).wait()
        return carry

    lax.fori_loop(0, 2, branch, 0)


@jax.jit
def pallas_concat_heads__gqa_block_cached__gqa_block_cached__near_ridge_kernel(
        A_x, A_k_cache, A_v_cache, A_wq, A_wo, B_x, B_k_cache, B_v_cache, B_wq, B_wo):
    hbm = pl.BlockSpec(memory_space=pl.ANY)
    out = pl.pallas_call(
        _kernel,
        out_shape=jax.ShapeDtypeStruct((M, 2 * D), jnp.bfloat16),
        in_specs=[hbm] * 10,
        out_specs=hbm,
        scratch_shapes=[
            pltpu.VMEM((2, B, D, SQ), jnp.bfloat16),
            pltpu.VMEM((M, D), jnp.bfloat16),
            pltpu.VMEM((2, D, HD), jnp.bfloat16),
            pltpu.VMEM((2, D, HD), jnp.bfloat16),
            pltpu.VMEM((2, B, HKV, SK, DH), jnp.bfloat16),
            pltpu.VMEM((2, B, HKV, SK, DH), jnp.bfloat16),
            pltpu.VMEM((M, HD), jnp.bfloat16),
            pltpu.VMEM((M, HD), jnp.bfloat16),
            pltpu.VMEM((2 * D, M), jnp.bfloat16),
            pltpu.VMEM((M, 2 * D), jnp.bfloat16),
            pltpu.SemaphoreType.DMA((2, 2)),
            pltpu.SemaphoreType.DMA((2,)),
            pltpu.SemaphoreType.DMA((2, N1)),
            pltpu.SemaphoreType.DMA((2,)),
            pltpu.SemaphoreType.DMA((2, N2)),
            pltpu.SemaphoreType.DMA((2, N2)),
            pltpu.SemaphoreType.DMA((2, N3)),
        ],
        compiler_params=pltpu.CompilerParams(vmem_limit_bytes=126 * 1024 * 1024),
    )(jnp.swapaxes(A_x, 1, 2), A_k_cache, A_v_cache, A_wq, A_wo.T,
      jnp.swapaxes(B_x, 1, 2), B_k_cache, B_v_cache, B_wq, B_wo.T)
    return out.reshape(B, SQ, 2 * D)
```
